```python
import jax
import jax.numpy as jnp

def _softmax(x, axis=-1):
    return jax.nn.softmax(x, axis=axis)
def _gelu(x):
    return jax.nn.gelu(x, approximate=True)
def _silu(x):
    return jax.nn.silu(x)
def _sigmoid(x):
    return jax.nn.sigmoid(x)
def _layernorm(x, axis=-1, eps=1e-5):
    m = jnp.mean(x, axis=axis, keepdims=True)
    v = jnp.var(x, axis=axis, keepdims=True)
    return (x - m) / jnp.sqrt(v + eps)
def _scatter_add(tgt, idx, src, axis=0):
    return tgt.at[idx].add(src)
def _segment_sum(src, seg, n):
    return jax.ops.segment_sum(src, seg, n)
class _Rng:
    def __init__(self, key):
        self._k = key
    def _next(self):
        self._k, sub = jax.random.split(self._k)
        return sub
    def normal(self, shape):
        return jax.random.normal(self._next(), shape, dtype=jnp.bfloat16)
    def randint(self, lo, hi, shape):
        return jax.random.randint(self._next(), shape, lo, hi, dtype=jnp.int32)
    def uniform(self, shape, lo=0.0, hi=1.0):
        return jax.random.uniform(self._next(), shape, jnp.bfloat16, lo, hi)
    def permutation(self, n):
        return jax.random.permutation(self._next(), n)


kernel_name = 'interleave_layers__sliding_local_dilated__spectral_gfnet__prompt'

def setup_inputs():
    _rng = _Rng(jax.random.key(int.from_bytes(__import__("os").urandom(4), "little")))
    _w = (lambda a: (lambda t: t.astype(jnp.bfloat16) if jnp.issubdtype(t.dtype, jnp.floating) else t)(jnp.asarray(a)))
    def _A_setup():
        B, S, D = 1, 2048, 1024
        return {
            "x": _w((lambda *s: _rng.normal(s) * 0.05)(B, S, D)),
            "wqkv": _w((lambda *s: _rng.normal(s) * 0.05)(D, 3 * D)),
            "wo": _w((lambda *s: _rng.normal(s) * 0.05)(D, D)),
        }
    _A_in = _A_setup()

    def _B_setup():
        B, S, D = 1, 2048, 1024
        Df = D // 2 + 1
        return {
            "x": _w((lambda *s: _rng.normal(s) * 0.05)(B, S, D)),
            "w_r": _w((lambda *s: _rng.normal(s) * 0.05)(S, Df) * 0.02),
            "w_i": _w((lambda *s: _rng.normal(s) * 0.05)(S, Df) * 0.02),
        }
    _B_in = _B_setup()

    return {
        "A_x": _A_in["x"],
        "A_wqkv": _A_in["wqkv"],
        "A_wo": _A_in["wo"],
        "B_x": _B_in["x"],
        "B_w_r": _B_in["w_r"],
        "B_w_i": _B_in["w_i"],
    }

def reference(A_x, A_wqkv, A_wo, B_x, B_w_r, B_w_i):
    def _A_ref(x, wqkv, wo):
        B, S, D = x.shape
        H = 32; Dh = D // H
        W, dil = 8, 2
        qkv = (lambda x, *d: x.transpose(*d))((x @ wqkv).reshape(B, S, 3, H, Dh), 2, 0, 3, 1, 4)
        q, k, v = qkv[0], qkv[1], qkv[2]
        scale = Dh ** -0.5
        pos = jnp.arange(S)
        off = jnp.arange(W) * dil
        idx = pos[:, None] - off[None, :]
        mask = idx >= 0
        idx_c = jnp.where(mask, idx, 0).reshape(-1)
        kg = k[:, :, idx_c, :].reshape(B, H, S, W, Dh)
        vg = v[:, :, idx_c, :].reshape(B, H, S, W, Dh)
        logits = jnp.einsum("bhsd,bhswd->bhsw", q, kg) * scale
        logits = jnp.where(mask[None, None, :, :], logits, -1e9)
        attn = _softmax(logits, axis=-1)
        o = jnp.einsum("bhsw,bhswd->bhsd", attn, vg)
        return (lambda x, *d: x.transpose(*d))(o, 0, 2, 1, 3).reshape(B, S, D) @ wo

    def _B_ref(x, w_r, w_i):
        B, S, D = x.shape
        X = (lambda x, axes=(-2,-1): jnp.fft.rfft2(x.astype(jnp.float32), axes=axes))(x, axes=(-2, -1))
        W = w_r + 1j * w_i
        X = X * W
        y = (lambda x, s, axes=(-2,-1): jnp.fft.irfft2(x, s=s, axes=axes).astype(jnp.bfloat16))(X, (S, D), axes=(-2, -1))
        return y

    x = A_x
    x = x + _A_ref(_layernorm(x, axis=-1), A_wqkv, A_wo)
    x = x + _B_ref(_layernorm(x, axis=-1), B_w_r, B_w_i)
    x = x + _A_ref(_layernorm(x, axis=-1), A_wqkv, A_wo)
    x = x + _B_ref(_layernorm(x, axis=-1), B_w_r, B_w_i)
    return x
```

```python
import functools
import numpy as np
import ml_dtypes
import jax
import jax.numpy as jnp
from jax import lax
import jax.experimental.pallas as pl
import jax.experimental.pallas.tpu as pltpu

S, D, H, DH, WIN, DIL = 2048, 1024, 32, 32, 8, 2
DF = D // 2 + 1
L = 128
NT = D // L
R = 16
PAD = 16
BM = 256
CH = 16
F32, BF16, U32 = jnp.float32, jnp.bfloat16, jnp.uint32
RS2 = float(np.sqrt(0.5))


def _consts():
    bf = ml_dtypes.bfloat16
    pq = np.zeros((L, L), np.float32)
    for hp in range(4):
        for t in range(8):
            for jj in range(2):
                for b in range(2):
                    pq[hp * 32 + t * 4 + jj * 2 + b, jj * 64 + t * 8 + hp * 2 + b] = 1
    head = (np.arange(L) % 64) // 2
    ones = (head[:, None] == head[None, :]).astype(np.float32)
    cls = [[l for l in range(L) if l % 4 == 0], [l for l in range(L) if l % 4 == 2],
           [l for l in range(L) if l % 8 in (1, 7)], [l for l in range(L) if l % 8 in (3, 5)]]
    pw = np.zeros((L, L), np.float32)
    for g in range(4):
        for i, l in enumerate(cls[g]):
            pw[l, g * 32 + i] = 1
    bfly = np.array(_split(list(np.eye(8))))
    fd = np.zeros((4, 2 * L, 2 * L))
    fi = np.zeros((4, 2 * L, 2 * L))
    d = np.arange(D)
    for g in range(4):
        ks = np.array([128 * s + l for s in range(4) for l in cls[g]])
        ang = 2 * np.pi * ((d[:, None] * ks[None, :]) % D) / D
        full = np.concatenate([np.cos(ang), -np.sin(ang)], 1)
        wt = np.full(2 * L, 2.0)
        if g == 0:
            full[:, L] = np.cos(np.pi * d)
            wt[0] = wt[L] = 1.0
        bt = np.kron(bfly[2 * g:2 * g + 2].T, np.eye(L))
        m = np.linalg.lstsq(bt, full, rcond=None)[0]
        assert np.abs(bt @ m - full).max() < 1e-9
        fd[g] = m
        fi[g] = (m * wt[None, :]).T / (S * D)
    n2 = np.arange(L)
    gf = np.zeros((R, 2 * L, 2 * L))
    for k1 in range(R):
        ang = 2 * np.pi * (((k1 + R * n2)[:, None] * n2[None, :]) % S) / S
        c, s = np.cos(ang), -np.sin(ang)
        gf[k1] = np.block([[c, -s], [s, c]])
    gi = gf.transpose(0, 2, 1)
    small = np.stack([pq, ones, pw])
    return (small.astype(bf), np.concatenate([fd, fi]).astype(bf),
            np.concatenate([gf, gi]).astype(bf))


def _split(z):
    a = [z[j] + z[j + 4] for j in range(4)]
    b = [z[j] - z[j + 4] for j in range(4)]
    p = (b[1] - b[3]) * RS2
    q = (b[1] + b[3]) * RS2
    return [a[0] + a[2], a[1] + a[3], a[0] - a[2], a[1] - a[3],
            b[0] + p, b[2] + q, b[0] - p, b[2] - q]


def _merge(y):
    a = [y[0] + y[2], y[1] + y[3], y[0] - y[2], y[1] - y[3]]
    p = (y[4] - y[6]) * RS2
    q = (y[5] - y[7]) * RS2
    b = [y[4] + y[6], p + q, y[5] + y[7], q - p]
    return [a[j] + b[j] for j in range(4)] + [a[j] - b[j] for j in range(4)]


def _tw(x, k, n, sgn):
    r, i = x
    k %= n
    if k == 0:
        return x
    if 4 * k == n:
        return (-i, r) if sgn > 0 else (i, -r)
    c, s = float(np.cos(2 * np.pi * k / n)), sgn * float(np.sin(2 * np.pi * k / n))
    if 8 * k == n or 8 * k == 3 * n:
        if (c > 0) == (s > 0):
            return ((r - i) * c, (r + i) * c)
        return ((r + i) * c, (i - r) * c)
    return (r * c - i * s, r * s + i * c)


def _fft4(x, sgn):
    (ar, ai), (br, bi), (cr, ci), (dr, di) = x
    pr, pi_, mr, mi = ar + cr, ai + ci, ar - cr, ai - ci
    qr, qi, nr, ni = br + dr, bi + di, br - dr, bi - di
    o1, o3 = (mr - ni, mi + nr), (mr + ni, mi - nr)
    if sgn < 0:
        o1, o3 = o3, o1
    return [(pr + qr, pi_ + qi), o1, (pr - qr, pi_ - qi), o3]


def _fft16(x, sgn):
    st = [_fft4([x[b + 4 * a] for a in range(4)], sgn) for b in range(4)]
    out = [None] * 16
    for ka in range(4):
        o = _fft4([_tw(st[b][ka], b * ka, 16, sgn) for b in range(4)], sgn)
        for kb in range(4):
            out[ka + 4 * kb] = o[kb]
    return out


def _ln(x):
    m = jnp.mean(x, axis=-1, keepdims=True)
    xc = x - m
    v = jnp.mean(xc * xc, axis=-1, keepdims=True)
    return xc * lax.rsqrt(v + 1e-5)


def _dot(a, b):
    return jnp.dot(a, b, preferred_element_type=F32)


def _block_transpose(tiles, g):
    n = len(tiles)
    lane = lax.broadcasted_iota(jnp.int32, tiles[0].shape, 1)
    st = 1
    while st < n:
        hi = (lane & (g * st)) != 0
        new = list(tiles)
        for a in range(n):
            if a & st == 0:
                b = a | st
                new[a] = jnp.where(hi, pltpu.roll(tiles[b], g * st, 1), tiles[a])
                new[b] = jnp.where(hi, tiles[b], pltpu.roll(tiles[a], L - g * st, 1))
        tiles = new
        st *= 2
    return tiles


def _lo(u):
    return pltpu.bitcast(u << 16, F32)


def _hi(u):
    return pltpu.bitcast(u & jnp.uint32(0xFFFF0000), F32)


def _kernel(x_hbm, wqkv_hbm, wo_hbm, wr_hbm, wi_hbm, small_hbm, fd_hbm, g_hbm, o_hbm,
            xs, hs, wq, wou, wop, wraw, wp, small, fd, gm, q0, k0, v0, q1, k1_, v1, us, ys, sems):
    qkv = ((q0, k0, v0), (q1, k1_, v1))
    srcs = [(small_hbm, small), (wqkv_hbm, wq), (x_hbm, hs), (wo_hbm, wop), (wr_hbm, wraw.at[0]),
            (wi_hbm, wraw.at[1]), (fd_hbm, fd), (g_hbm, gm)]
    cps = [pltpu.make_async_copy(a, b, sems.at[i]) for i, (a, b) in enumerate(srcs)]
    for c in cps:
        c.start()
    cps[0].wait()
    cps[1].wait()

    def perm_wq(i, _):
        rows = pl.ds(pl.multiple_of(i * 128, 128), 128)
        for m in range(3):
            t = [pltpu.bitcast(_dot(wq[rows, m * D + s * L:m * D + (s + 1) * L], small[0]).astype(BF16), U32)
                 for s in range(NT)]
            t = _block_transpose(t, 8)
            for s in range(NT):
                wq[rows, m * D + s * L:m * D + (s + 1) * L] = pltpu.bitcast(t[s], BF16)
        return _
    with jax.named_scope('perm_wq'):
        lax.fori_loop(0, D // 128, perm_wq, None)

    cps[2].wait()

    cps[3].wait()
    for c in range(NT):
        wou[c] = pltpu.bitcast(wop[:, c * L:(c + 1) * L], U32)
    for t in range(NT):
        for jj in range(2):
            wop[t * L + jj * 64:t * L + jj * 64 + 64, :] = pltpu.bitcast(
                jnp.concatenate([wou[c, pl.ds(t * 2 + jj, 32, stride=16), :] for c in range(NT)], 1), BF16)

    scale = DH ** -0.5

    def attn_layer(first):
        def proj(i, sl):
            rows = pl.ds(pl.multiple_of(i * BM, BM), BM)
            h = hs[rows, :]
            if first:
                x = h.astype(F32)
                xs[rows, :] = x
                h = _ln(x).astype(BF16)
            q, k, v = qkv[sl]
            for m, dst in enumerate((q, k, v)):
                r = _dot(h, wq[:, m * D:(m + 1) * D])
                off = PAD if m else 0
                for t in range(NT):
                    dst[t, off:off + BM, :] = r[:, t * L:(t + 1) * L]

        def attn(i, sl):
            r0 = pl.multiple_of(i * BM, BM)
            rows = pl.ds(r0, BM)
            qs, ks, vs = qkv[sl]
            part = []
            for w in range(WIN):
                acc = None
                for t in range(NT):
                    pr = qs[t] * ks[t, PAD - DIL * w:PAD - DIL * w + BM, :]
                    acc = pr if acc is None else acc + pr
                part.append(acc.astype(BF16))
            lg = _dot(jnp.concatenate(part, 0), small[1]) * scale
            pos = r0 + lax.broadcasted_iota(jnp.int32, (BM, L), 0)
            lg = [jnp.where(pos >= DIL * w, lg[w * BM:(w + 1) * BM], -1e9) for w in range(WIN)]
            mx = functools.reduce(jnp.maximum, lg)
            e = [jnp.exp(l - mx) for l in lg]
            inv = 1.0 / functools.reduce(jnp.add, e)
            p = [a * inv for a in e]
            o = []
            for t in range(NT):
                acc = None
                for w in range(WIN):
                    pr = p[w] * vs[t, PAD - DIL * w:PAD - DIL * w + BM, :]
                    acc = pr if acc is None else acc + pr
                o.append(acc.astype(BF16))
            qkv[1 - sl][1][:, 0:PAD, :] = ks[:, BM:BM + PAD, :]
            qkv[1 - sl][2][:, 0:PAD, :] = vs[:, BM:BM + PAD, :]
            xs[rows, :] = xs[rows, :] + _dot(jnp.concatenate(o, 1), wop[...])

        def body(j, _):
            for sl in range(2):
                proj(2 * j + sl + 1, 1 - sl)
                attn(2 * j + sl, sl)
            return _
        nb = S // BM
        qkv[0][1][:, 0:PAD, :] = jnp.zeros((NT, PAD, L), F32)
        qkv[0][2][:, 0:PAD, :] = jnp.zeros((NT, PAD, L), F32)
        proj(0, 0)
        with jax.named_scope('abody'):
            lax.fori_loop(0, nb // 2 - 1, body, None)
        proj(nb - 1, 1)
        attn(nb - 2, 0)
        attn(nb - 1, 1)

    def prep_w():
        def body(i, _):
            rows = pl.ds(pl.multiple_of(i * 256, 256), 256)
            urows = pl.ds(pl.multiple_of(i * 128, 128), 128)
            for c in range(2):
                t = [pltpu.bitcast(lax.dot_general(wraw[c, s * L:(s + 1) * L, rows], small[2], (((0,), (0,)), ((), ())),
                                                   preferred_element_type=F32).astype(BF16), U32)
                     for s in range(4)]
                t = _block_transpose(t, 32)
                for s in range(4):
                    wp[c, s, urows, :] = t[s]
                ny = jnp.broadcast_to(wraw[c, 4 * L:DF, rows].astype(F32), (L, 256)).T
                wp[c, 4, urows, :] = pltpu.bitcast(ny.astype(BF16), U32)
            return _
        with jax.named_scope('body'):
            lax.fori_loop(0, S // 256, body, None)

    lane0 = lax.broadcasted_iota(jnp.int32, (8, L), 1) == 0

    def spec_layer(last):
        def fwd(c, _):
            c0 = pl.multiple_of(c * CH, CH)
            x = jnp.concatenate([xs[pl.ds(n * L + c0, CH), :] for n in range(R)], 0)
            z = _ln(x)
            sp = _split([z[:, t * L:(t + 1) * L] for t in range(NT)])
            for g in range(4):
                u = _dot(jnp.concatenate([sp[2 * g], sp[2 * g + 1]], 1).astype(BF16), fd[g])
                for tile in ((g, 4) if g == 0 else (g,)):
                    res = []
                    for hf in range(CH // 8):
                        xin = []
                        for n in range(R):
                            re = u[n * CH + hf * 8:n * CH + hf * 8 + 8, 0:L]
                            im = u[n * CH + hf * 8:n * CH + hf * 8 + 8, L:2 * L]
                            if tile == 0:
                                im = jnp.where(lane0, 0.0, im)
                            if tile == 4:
                                re, im = jnp.where(lane0, im, 0.0), jnp.zeros((8, L), F32)
                            xin.append((re, im))
                        res.append(_fft16(xin, -1))
                    for k1 in range(R):
                        for ri in range(2):
                            us[k1, pl.ds(ri * L + c0, CH), tile * L:(tile + 1) * L] = jnp.concatenate(
                                [r_[k1][ri] for r_ in res], 0).astype(BF16)
            return _
        with jax.named_scope('fwd'):
            lax.fori_loop(0, L // CH, fwd, None)

        def mid(j, _):
            w = [[wp[c, t, pl.ds(j, L, stride=R // 2), :] for t in range(5)] for c in range(2)]
            for par, f in enumerate((_lo, _hi)):
                k1 = 2 * j + par
                xf = _dot(gm[k1], us[k1])
                wr = jnp.concatenate([f(a) for a in w[0]], 1)
                wi = jnp.concatenate([f(a) for a in w[1]], 1)
                xr, xi = xf[0:L], xf[L:2 * L]
                y = jnp.concatenate([xr * wr - xi * wi, xr * wi + xi * wr], 0).astype(BF16)
                ys[k1] = _dot(gm[R + k1], y)
            return _
        with jax.named_scope('mid'):
            lax.fori_loop(0, R // 2, mid, None)

        def inv(c, _):
            c0 = pl.multiple_of(c * CH, CH)
            yt = []
            for g in range(4):
                re, im = [], []
                for hf in range(CH // 8):
                    ld = lambda t: [(ys[k1, pl.ds(c0 + hf * 8, 8), t * L:(t + 1) * L],
                                     ys[k1, pl.ds(L + c0 + hf * 8, 8), t * L:(t + 1) * L]) for k1 in range(R)]
                    o = _fft16(ld(g), 1)
                    if g == 0:
                        o4 = _fft16(ld(4), 1)
                        o = [(a[0], jnp.where(lane0, b[0], a[1])) for a, b in zip(o, o4)]
                    re.append([a[0] for a in o])
                    im.append([a[1] for a in o])
                lhs = jnp.concatenate(
                    [jnp.concatenate([pt[hf][n] for n in range(R) for hf in range(CH // 8)], 0).astype(BF16)
                     for pt in (re, im)], 1)
                r = _dot(lhs, fd[4 + g])
                yt += [r[:, 0:L], r[:, L:2 * L]]
            y = jnp.concatenate(_merge(yt), 1)
            for n in range(R):
                rows = pl.ds(n * L + c0, CH)
                xn = xs[rows, :] + y[n * CH:(n + 1) * CH]
                if last:
                    hs[rows, :] = xn.astype(BF16)
                else:
                    xs[rows, :] = xn
                    hs[rows, :] = _ln(xn).astype(BF16)
            return _
        with jax.named_scope('inv'):
            lax.fori_loop(0, L // CH, inv, None)

    attn_layer(True)
    for c in cps[4:]:
        c.wait()
    prep_w()
    spec_layer(False)
    attn_layer(False)
    spec_layer(True)
    out = pltpu.make_async_copy(hs, o_hbm, sems.at[0])
    out.start()
    out.wait()


_SMALL, _FD, _GM = _consts()


@jax.jit
def pallas_interleave_layers__sliding_local_dilated__spectral_gfnet__prompt_kernel(
    A_x: jax.Array,
    A_wqkv: jax.Array,
    A_wo: jax.Array,
    B_x: jax.Array,
    B_w_r: jax.Array,
    B_w_i: jax.Array,
):
    del B_x
    V = pltpu.VMEM
    out = pl.pallas_call(
        _kernel,
        in_specs=[pl.BlockSpec(memory_space=pltpu.HBM)] * 8,
        out_specs=pl.BlockSpec(memory_space=pl.ANY),
        out_shape=jax.ShapeDtypeStruct((S, D), BF16),
        scratch_shapes=[
            V((S, D), F32), V((S, D), BF16), V((D, 3 * D), BF16), V((NT, D // 2, L), U32), V((D, D), BF16),
            V((2, DF, S), BF16), V((2, 5, S // 2, L), U32), V(_SMALL.shape, BF16), V(_FD.shape, BF16),
            V(_GM.shape, BF16), V((NT, BM, L), F32), V((NT, BM + PAD, L), F32), V((NT, BM + PAD, L), F32),
            V((NT, BM, L), F32), V((NT, BM + PAD, L), F32), V((NT, BM + PAD, L), F32),
            V((R, 2 * L, 5 * L), BF16), V((R, 2 * L, 5 * L), F32), pltpu.SemaphoreType.DMA((8,)),
        ],
        compiler_params=pltpu.CompilerParams(vmem_limit_bytes=110 * 1024 * 1024),
    )(A_x.reshape(S, D), A_wqkv, A_wo, B_w_r.T, B_w_i.T, _SMALL, _FD, _GM)
    return out.reshape(1, S, D)
```

```python
import functools
import numpy as np
import ml_dtypes
import jax
import jax.numpy as jnp
from jax import lax
import jax.experimental.pallas as pl
import jax.experimental.pallas.tpu as pltpu

S, D, H, DH, WIN, DIL = 2048, 1024, 32, 32, 8, 2
DF = D // 2 + 1
L = 128
NT = D // L
R = 16
PAD = 16
BM = 512
CH = 16
F32, BF16, U32 = jnp.float32, jnp.bfloat16, jnp.uint32
RS2 = float(np.sqrt(0.5))


def _consts():
    bf = ml_dtypes.bfloat16
    pq = np.zeros((L, L), np.float32)
    for hp in range(4):
        for t in range(8):
            for jj in range(2):
                for b in range(2):
                    pq[hp * 32 + t * 4 + jj * 2 + b, jj * 64 + t * 8 + hp * 2 + b] = 1
    head = (np.arange(L) % 64) // 2
    ones = (head[:, None] == head[None, :]).astype(np.float32)
    cls = [[l for l in range(L) if l % 4 == 0], [l for l in range(L) if l % 4 == 2],
           [l for l in range(L) if l % 8 in (1, 7)], [l for l in range(L) if l % 8 in (3, 5)]]
    pw = np.zeros((L, L), np.float32)
    for g in range(4):
        for i, l in enumerate(cls[g]):
            pw[l, g * 32 + i] = 1
    bfly = np.array(_split(list(np.eye(8))))
    fd = np.zeros((4, 2 * L, 2 * L))
    fi = np.zeros((4, 2 * L, 2 * L))
    d = np.arange(D)
    for g in range(4):
        ks = np.array([128 * s + l for s in range(4) for l in cls[g]])
        ang = 2 * np.pi * ((d[:, None] * ks[None, :]) % D) / D
        full = np.concatenate([np.cos(ang), -np.sin(ang)], 1)
        wt = np.full(2 * L, 2.0)
        if g == 0:
            full[:, L] = np.cos(np.pi * d)
            wt[0] = wt[L] = 1.0
        bt = np.kron(bfly[2 * g:2 * g + 2].T, np.eye(L))
        m = np.linalg.lstsq(bt, full, rcond=None)[0]
        assert np.abs(bt @ m - full).max() < 1e-9
        fd[g] = m
        fi[g] = (m * wt[None, :]).T / (S * D)
    n2 = np.arange(L)
    gf = np.zeros((R, 2 * L, 2 * L))
    for k1 in range(R):
        ang = 2 * np.pi * (((k1 + R * n2)[:, None] * n2[None, :]) % S) / S
        c, s = np.cos(ang), -np.sin(ang)
        gf[k1] = np.block([[c, -s], [s, c]])
    gi = gf.transpose(0, 2, 1)
    small = np.stack([pq, ones, pw])
    return (small.astype(bf), np.concatenate([fd, fi]).astype(bf),
            np.concatenate([gf, gi]).astype(bf))


def _split(z):
    a = [z[j] + z[j + 4] for j in range(4)]
    b = [z[j] - z[j + 4] for j in range(4)]
    p = (b[1] - b[3]) * RS2
    q = (b[1] + b[3]) * RS2
    return [a[0] + a[2], a[1] + a[3], a[0] - a[2], a[1] - a[3],
            b[0] + p, b[2] + q, b[0] - p, b[2] - q]


def _merge(y):
    a = [y[0] + y[2], y[1] + y[3], y[0] - y[2], y[1] - y[3]]
    p = (y[4] - y[6]) * RS2
    q = (y[5] - y[7]) * RS2
    b = [y[4] + y[6], p + q, y[5] + y[7], q - p]
    return [a[j] + b[j] for j in range(4)] + [a[j] - b[j] for j in range(4)]


def _tw(x, k, n, sgn):
    r, i = x
    k %= n
    if k == 0:
        return x
    if 4 * k == n:
        return (-i, r) if sgn > 0 else (i, -r)
    c, s = float(np.cos(2 * np.pi * k / n)), sgn * float(np.sin(2 * np.pi * k / n))
    if 8 * k == n or 8 * k == 3 * n:
        if (c > 0) == (s > 0):
            return ((r - i) * c, (r + i) * c)
        return ((r + i) * c, (i - r) * c)
    return (r * c - i * s, r * s + i * c)


def _fft4(x, sgn):
    (ar, ai), (br, bi), (cr, ci), (dr, di) = x
    pr, pi_, mr, mi = ar + cr, ai + ci, ar - cr, ai - ci
    qr, qi, nr, ni = br + dr, bi + di, br - dr, bi - di
    o1, o3 = (mr - ni, mi + nr), (mr + ni, mi - nr)
    if sgn < 0:
        o1, o3 = o3, o1
    return [(pr + qr, pi_ + qi), o1, (pr - qr, pi_ - qi), o3]


def _fft16(x, sgn):
    st = [_fft4([x[b + 4 * a] for a in range(4)], sgn) for b in range(4)]
    out = [None] * 16
    for ka in range(4):
        o = _fft4([_tw(st[b][ka], b * ka, 16, sgn) for b in range(4)], sgn)
        for kb in range(4):
            out[ka + 4 * kb] = o[kb]
    return out


def _ln(x):
    m = jnp.mean(x, axis=-1, keepdims=True)
    xc = x - m
    v = jnp.mean(xc * xc, axis=-1, keepdims=True)
    return xc * lax.rsqrt(v + 1e-5)


def _dot(a, b):
    return jnp.dot(a, b, preferred_element_type=F32)


def _block_transpose(tiles, g):
    n = len(tiles)
    lane = lax.broadcasted_iota(jnp.int32, tiles[0].shape, 1)
    st = 1
    while st < n:
        hi = (lane & (g * st)) != 0
        new = list(tiles)
        for a in range(n):
            if a & st == 0:
                b = a | st
                new[a] = jnp.where(hi, pltpu.roll(tiles[b], g * st, 1), tiles[a])
                new[b] = jnp.where(hi, tiles[b], pltpu.roll(tiles[a], L - g * st, 1))
        tiles = new
        st *= 2
    return tiles


def mix(*gens):
    gens = list(gens)
    while gens:
        gens = [g for g in gens if next(g, 0) is None]


def _lo(u):
    return pltpu.bitcast(u << 16, F32)


def _hi(u):
    return pltpu.bitcast(u & jnp.uint32(0xFFFF0000), F32)


def _kernel(x_hbm, wqkv_hbm, wo_hbm, wr_hbm, wi_hbm, small_hbm, fd_hbm, g_hbm, o_hbm,
            xs, hs, wq, wou, wop, wraw, wp, small, fd, gm, q0, k0, v0, q1, k1_, v1, us, ys, sems):
    qkv = ((q0, k0, v0), (q1, k1_, v1))
    srcs = [(small_hbm, small), (wqkv_hbm, wq), (x_hbm, hs), (wo_hbm, wop), (wr_hbm, wraw.at[0]),
            (wi_hbm, wraw.at[1]), (fd_hbm, fd), (g_hbm, gm)]
    cps = [pltpu.make_async_copy(a, b, sems.at[i]) for i, (a, b) in enumerate(srcs)]

    def wq_cp(i):
        rows = pl.ds(pl.multiple_of(i * 128, 128), 128)
        return pltpu.make_async_copy(wqkv_hbm.at[rows], wq.at[rows], sems.at[8 + i])
    cps[0].start()
    for i in range(3):
        wq_cp(i).start()
    cps[0].wait()

    def perm_wq(i, _):
        wq_cp(i).wait()

        @pl.when(i + 3 < D // 128)
        def _start_next():
            wq_cp(i + 3).start()

        @pl.when(i == 4)
        def _start_more():
            cps[2].start()
            cps[3].start()
        rows = pl.ds(pl.multiple_of(i * 128, 128), 128)
        for m in range(3):
            t = [pltpu.bitcast(_dot(wq[rows, m * D + s * L:m * D + (s + 1) * L], small[0]).astype(BF16), U32)
                 for s in range(NT)]
            t = _block_transpose(t, 8)
            for s in range(NT):
                wq[rows, m * D + s * L:m * D + (s + 1) * L] = pltpu.bitcast(t[s], BF16)
        return _
    with jax.named_scope('perm_wq'):
        lax.fori_loop(0, D // 128, perm_wq, None)

    cps[2].wait()

    cps[3].wait()
    for c in cps[4:]:
        c.start()
    for c in range(NT):
        wou[c] = pltpu.bitcast(wop[:, c * L:(c + 1) * L], U32)
    for t in range(NT):
        for jj in range(2):
            wop[t * L + jj * 64:t * L + jj * 64 + 64, :] = pltpu.bitcast(
                jnp.concatenate([wou[c, pl.ds(t * 2 + jj, 32, stride=16), :] for c in range(NT)], 1), BF16)

    scale = DH ** -0.5

    def attn_layer(first):
        def proj(i, sl):
            rows = pl.ds(pl.multiple_of(i * BM, BM), BM)
            h = hs[rows, :]
            if first:
                x = h.astype(F32)
                xs[rows, :] = x
                h = _ln(x).astype(BF16)
            q, k, v = qkv[sl]
            for m, dst in enumerate((q, k, v)):
                off = PAD if m else 0
                for t in range(NT):
                    dst[t, off:off + BM, :] = _dot(h, wq[:, m * D + t * L:m * D + (t + 1) * L])
                    yield

        def attn(i, sl):
            r0 = pl.multiple_of(i * BM, BM)
            rows = pl.ds(r0, BM)
            qs, ks, vs = qkv[sl]
            part = []
            for w in range(WIN):
                acc = None
                for t in range(NT):
                    pr = qs[t] * ks[t, PAD - DIL * w:PAD - DIL * w + BM, :]
                    acc = pr if acc is None else acc + pr
                part.append(acc.astype(BF16))
                yield
            lg = _dot(jnp.concatenate(part, 0), small[1]) * scale
            yield
            yield
            pos = r0 + lax.broadcasted_iota(jnp.int32, (BM, L), 0)
            lg = [jnp.where(pos >= DIL * w, lg[w * BM:(w + 1) * BM], -1e9) for w in range(WIN)]
            mx = functools.reduce(jnp.maximum, lg)
            yield
            yield
            e = [jnp.exp(l - mx) for l in lg]
            inv = 1.0 / functools.reduce(jnp.add, e)
            p = [a * inv for a in e]
            yield
            yield
            o = []
            for t in range(NT):
                acc = None
                for w in range(WIN):
                    pr = p[w] * vs[t, PAD - DIL * w:PAD - DIL * w + BM, :]
                    acc = pr if acc is None else acc + pr
                o.append(acc.astype(BF16))
                yield
            yield
            yield
            yield
            qkv[1 - sl][1][:, 0:PAD, :] = ks[:, BM:BM + PAD, :]
            qkv[1 - sl][2][:, 0:PAD, :] = vs[:, BM:BM + PAD, :]
            xs[rows, :] = xs[rows, :] + _dot(jnp.concatenate(o, 1), wop[...])

        def body(j, _):
            for sl in range(2):
                mix(proj(2 * j + sl + 1, 1 - sl), attn(2 * j + sl, sl))
            return _
        nb = S // BM
        qkv[0][1][:, 0:PAD, :] = jnp.zeros((NT, PAD, L), F32)
        qkv[0][2][:, 0:PAD, :] = jnp.zeros((NT, PAD, L), F32)
        mix(proj(0, 0))
        with jax.named_scope('abody'):
            lax.fori_loop(0, nb // 2 - 1, body, None)
        if first:
            for c in cps[4:]:
                c.wait()
        mix(proj(nb - 1, 1), attn(nb - 2, 0), *([prep_w()] if first else []))
        mix(attn(nb - 1, 1))

    def prep_w():
        for i in range(S // 256):
            rows = pl.ds(i * 256, 256)
            urows = pl.ds(i * 128, 128)
            for c in range(2):
                t = [pltpu.bitcast(lax.dot_general(wraw[c, s * L:(s + 1) * L, rows], small[2], (((0,), (0,)), ((), ())),
                                                   preferred_element_type=F32).astype(BF16), U32)
                     for s in range(4)]
                t = _block_transpose(t, 32)
                for s in range(4):
                    wp[c, s, urows, :] = t[s]
                ny = jnp.broadcast_to(wraw[c, 4 * L:DF, rows].astype(F32), (L, 256)).T
                wp[c, 4, urows, :] = pltpu.bitcast(ny.astype(BF16), U32)
                yield

    lane0 = lax.broadcasted_iota(jnp.int32, (8, L), 1) == 0

    def spec_layer(last):
        def fwd(c, _):
            c0 = pl.multiple_of(c * CH, CH)
            x = jnp.concatenate([xs[pl.ds(n * L + c0, CH), :] for n in range(R)], 0)
            z = _ln(x)
            sp = _split([z[:, t * L:(t + 1) * L] for t in range(NT)])
            for g in range(4):
                u = _dot(jnp.concatenate([sp[2 * g], sp[2 * g + 1]], 1).astype(BF16), fd[g])
                for tile in ((g, 4) if g == 0 else (g,)):
                    res = []
                    for hf in range(CH // 8):
                        xin = []
                        for n in range(R):
                            re = u[n * CH + hf * 8:n * CH + hf * 8 + 8, 0:L]
                            im = u[n * CH + hf * 8:n * CH + hf * 8 + 8, L:2 * L]
                            if tile == 0:
                                im = jnp.where(lane0, 0.0, im)
                            if tile == 4:
                                re, im = jnp.where(lane0, im, 0.0), jnp.zeros((8, L), F32)
                            xin.append((re, im))
                        res.append(_fft16(xin, -1))
                    for k1 in range(R):
                        for ri in range(2):
                            us[k1, pl.ds(ri * L + c0, CH), tile * L:(tile + 1) * L] = jnp.concatenate(
                                [r_[k1][ri] for r_ in res], 0).astype(BF16)
            return _
        with jax.named_scope('fwd'):
            lax.fori_loop(0, L // CH, fwd, None, unroll=2)

        def mid(j, _):
            w = [[wp[c, t, pl.ds(j, L, stride=R // 2), :] for t in range(5)] for c in range(2)]
            for par, f in enumerate((_lo, _hi)):
                k1 = 2 * j + par
                xf = _dot(gm[k1], us[k1])
                wr = jnp.concatenate([f(a) for a in w[0]], 1)
                wi = jnp.concatenate([f(a) for a in w[1]], 1)
                xr, xi = xf[0:L], xf[L:2 * L]
                y = jnp.concatenate([xr * wr - xi * wi, xr * wi + xi * wr], 0).astype(BF16)
                ys[k1] = _dot(gm[R + k1], y)
            return _
        with jax.named_scope('mid'):
            lax.fori_loop(0, R // 2, mid, None)

        def inv(c, _):
            c0 = pl.multiple_of(c * CH, CH)
            yt = []
            for g in range(4):
                re, im = [], []
                for hf in range(CH // 8):
                    ld = lambda t: [(ys[k1, pl.ds(c0 + hf * 8, 8), t * L:(t + 1) * L],
                                     ys[k1, pl.ds(L + c0 + hf * 8, 8), t * L:(t + 1) * L]) for k1 in range(R)]
                    o = _fft16(ld(g), 1)
                    if g == 0:
                        o4 = _fft16(ld(4), 1)
                        o = [(a[0], jnp.where(lane0, b[0], a[1])) for a, b in zip(o, o4)]
                    re.append([a[0] for a in o])
                    im.append([a[1] for a in o])
                lhs = jnp.concatenate(
                    [jnp.concatenate([pt[hf][n] for n in range(R) for hf in range(CH // 8)], 0).astype(BF16)
                     for pt in (re, im)], 1)
                r = _dot(lhs, fd[4 + g])
                yt += [r[:, 0:L], r[:, L:2 * L]]
            y = jnp.concatenate(_merge(yt), 1)
            for n in range(R):
                rows = pl.ds(n * L + c0, CH)
                xn = xs[rows, :] + y[n * CH:(n + 1) * CH]
                if last:
                    hs[rows, :] = xn.astype(BF16)
                else:
                    xs[rows, :] = xn
                    hs[rows, :] = _ln(xn).astype(BF16)
            if last:
                for n in range(R):
                    rows = pl.ds(n * L + c0, CH)
                    pltpu.make_async_copy(hs.at[rows], o_hbm.at[rows], sems.at[0]).start()
            return _
        with jax.named_scope('inv'):
            lax.fori_loop(0, L // CH, inv, None)

    attn_layer(True)
    spec_layer(False)
    attn_layer(False)
    spec_layer(True)
    out = pltpu.make_async_copy(hs, o_hbm, sems.at[0])
    out.wait()


_SMALL, _FD, _GM = _consts()


@jax.jit
def pallas_interleave_layers__sliding_local_dilated__spectral_gfnet__prompt_kernel(
    A_x: jax.Array,
    A_wqkv: jax.Array,
    A_wo: jax.Array,
    B_x: jax.Array,
    B_w_r: jax.Array,
    B_w_i: jax.Array,
):
    del B_x
    V = pltpu.VMEM
    out = pl.pallas_call(
        _kernel,
        in_specs=[pl.BlockSpec(memory_space=pltpu.HBM)] * 8,
        out_specs=pl.BlockSpec(memory_space=pl.ANY),
        out_shape=jax.ShapeDtypeStruct((S, D), BF16),
        scratch_shapes=[
            V((S, D), F32), V((S, D), BF16), V((D, 3 * D), BF16), V((NT, D // 2, L), U32), V((D, D), BF16),
            V((2, DF, S), BF16), V((2, 5, S // 2, L), U32), V(_SMALL.shape, BF16), V(_FD.shape, BF16),
            V(_GM.shape, BF16), V((NT, BM, L), F32), V((NT, BM + PAD, L), F32), V((NT, BM + PAD, L), F32),
            V((NT, BM, L), F32), V((NT, BM + PAD, L), F32), V((NT, BM + PAD, L), F32),
            V((R, 2 * L, 5 * L), BF16), V((R, 2 * L, 5 * L), F32), pltpu.SemaphoreType.DMA((16,)),
        ],
        compiler_params=pltpu.CompilerParams(vmem_limit_bytes=110 * 1024 * 1024),
    )(A_x.reshape(S, D), A_wqkv, A_wo, B_w_r.T, B_w_i.T, _SMALL, _FD, _GM)
    return out.reshape(1, S, D)
```
